```python
import jax
import jax.numpy as jnp

def _softmax(x, axis=-1):
    return jax.nn.softmax(x, axis=axis)
def _gelu(x):
    return jax.nn.gelu(x, approximate=True)
def _silu(x):
    return jax.nn.silu(x)
def _sigmoid(x):
    return jax.nn.sigmoid(x)
def _layernorm(x, axis=-1, eps=1e-5):
    m = jnp.mean(x, axis=axis, keepdims=True)
    v = jnp.var(x, axis=axis, keepdims=True)
    return (x - m) / jnp.sqrt(v + eps)
def _scatter_add(tgt, idx, src, axis=0):
    return tgt.at[idx].add(src)
def _segment_sum(src, seg, n):
    return jax.ops.segment_sum(src, seg, n)
class _Rng:
    def __init__(self, key):
        self._k = key
    def _next(self):
        self._k, sub = jax.random.split(self._k)
        return sub
    def normal(self, shape):
        return jax.random.normal(self._next(), shape, dtype=jnp.bfloat16)
    def randint(self, lo, hi, shape):
        return jax.random.randint(self._next(), shape, lo, hi, dtype=jnp.int32)
    def uniform(self, shape, lo=0.0, hi=1.0):
        return jax.random.uniform(self._next(), shape, jnp.bfloat16, lo, hi)
    def permutation(self, n):
        return jax.random.permutation(self._next(), n)


kernel_name = 'recurrent_scan__sliding_block_cached__moe_arch_mod__decode'

def setup_inputs():
    _rng = _Rng(jax.random.key(int.from_bytes(__import__("os").urandom(4), "little")))
    _w = (lambda a: (lambda t: t.astype(jnp.bfloat16) if jnp.issubdtype(t.dtype, jnp.floating) else t)(jnp.asarray(a)))
    def _A_setup():
        B, Sq, D = 1, 1, 512
        Hq, Hkv, Sk, Dh = 32, 32, 32768, 128
        assert Hq % Hkv == 0, (Hq, Hkv)
        return {
            "x": _w((lambda *s: _rng.normal(s) * 0.05)(B, Sq, D)),
            "k_cache": _w((lambda *s: _rng.normal(s) * 0.05)(B, Hkv, Sk, Dh)),
            "v_cache": _w((lambda *s: _rng.normal(s) * 0.05)(B, Hkv, Sk, Dh)),
            "wq": _w((lambda *s: _rng.normal(s) * 0.05)(D, Hq * Dh) * (D ** -0.5)),
            "wo": _w((lambda *s: _rng.normal(s) * 0.05)(Hq * Dh, D) * ((Hq * Dh) ** -0.5)),
        }
    _A_in = _A_setup()

    def _B_setup():
        B, S, D, F, C = 1, 1, 512, 1376, 1
        return {
            "x": _w((lambda *s: _rng.normal(s) * 0.05)(B, S, D)),
            "w_r": _w((lambda *s: _rng.normal(s) * 0.05)(D)),
            "w_gate": _w((lambda *s: _rng.normal(s) * 0.05)(D, F)),
            "w_up": _w((lambda *s: _rng.normal(s) * 0.05)(D, F)),
            "w_down": _w((lambda *s: _rng.normal(s) * 0.05)(F, D)),
        }
    _B_in = _B_setup()

    return {
        "A_x": _A_in["x"],
        "A_k_cache": _A_in["k_cache"],
        "A_v_cache": _A_in["v_cache"],
        "A_wq": _A_in["wq"],
        "A_wo": _A_in["wo"],
        "B_x": _B_in["x"],
        "B_w_r": _B_in["w_r"],
        "B_w_gate": _B_in["w_gate"],
        "B_w_up": _B_in["w_up"],
        "B_w_down": _B_in["w_down"],
    }

def reference(A_x, A_k_cache, A_v_cache, A_wq, A_wo, B_x, B_w_r, B_w_gate, B_w_up, B_w_down):
    def _A_ref(x, k_cache, v_cache, wq, wo):
        B, Sq, D = x.shape
        Hq, Dh = 32, 128
        Hkv, Sk = k_cache.shape[1], k_cache.shape[2]
        W = min(4096, max(256, Sk // 4))
        rep = Hq // Hkv
        q = (lambda x, *d: x.transpose(*d))((x @ wq).reshape(B, Sq, Hq, Dh), 0, 2, 1, 3)
        k = jnp.repeat(k_cache[:, :, Sk - W:, :], rep, axis=1)
        v = jnp.repeat(v_cache[:, :, Sk - W:, :], rep, axis=1)
        scores = jnp.einsum("bhqd,bhkd->bhqk", q, k) * (Dh ** -0.5)
        p = _softmax(scores, axis=-1)
        o = jnp.einsum("bhqk,bhkd->bhqd", p, v)
        return (lambda x, *d: x.transpose(*d))(o, 0, 2, 1, 3).reshape(B, Sq, Hq * Dh) @ wo

    def _B_ref(x, w_r, w_gate, w_up, w_down):
        B, S, D = x.shape
        C = 1
        r = x @ w_r
        idx = jnp.argsort(-r, axis=-1)[:, :C]
        idx_e = jnp.repeat(idx.reshape(B, C, 1), D, axis=2)
        x_sel = jnp.take_along_axis(x, idx_e, axis=1)
        g = _silu(x_sel @ w_gate)
        u = x_sel @ w_up
        y = (g * u) @ w_down
        r_sel = _sigmoid(jnp.take_along_axis(r, idx, axis=1))
        y = y * r_sel.reshape(B, C, 1)
        b_off = (jnp.arange(B) * S).reshape(B, 1)
        flat_idx = (idx + b_off).reshape(B * C)
        zero = (x * 0.0).reshape(B * S, D)
        upd = _scatter_add(zero, flat_idx, y.reshape(B * C, D), axis=0)
        return x + upd.reshape(B, S, D)

    x = A_x
    xn = _layernorm(x, axis=-1)
    s = _A_ref(xn, A_k_cache, A_v_cache, A_wq, A_wo)
    g = _silu(_B_ref(xn, B_w_r, B_w_gate, B_w_up, B_w_down))
    return x + s * g
```

```python
import jax
import jax.numpy as jnp
import jax.experimental.pallas as pl
import jax.experimental.pallas.tpu as pltpu

D = 512
NH = 32
DH = 128
SK = 32768
W = min(4096, max(256, SK // 4))
F = 1376

G = 8
NG = NH // G
CR = 64
RG = W // CR
NR = NG * RG
RPS = 4
NS = NR // RPS
SPG = RG // RPS
KS = RPS * CR
NW = F // 32
QO = G * DH
LATE = QO - 16 * NW
AHEAD = 6
LAG = 2
RING = 8
TINY = 8
VPU = (80, 32, 16)

BF16 = jnp.bfloat16
F32 = jnp.float32
_NT = (((1,), (1,)), ((), ()))
HI, LO = 0, 1
ds = pl.ds


def _late_blocks():
    blocks, r1 = [], LATE
    while r1 > DH:
        r0 = (r1 - 1) // DH * DH
        blocks.append((0, NG, r0, r1 - r0))
        r1 = r0
    blocks += [(2, 2, 0, DH), (1, 1, 0, DH)]
    r0 = 0
    for n in VPU:
        blocks.append((0, 1, r0, n))
        r0 += n
    assert r0 == DH
    return blocks


def _kernel(x_h, k_h, v_h, wq_h, wo_h, wr_h, wg_h, wu_h, wd_h, out_ref,
            x_v, wr_v, wq_v, kv_v, wo_v, wg_v, wu_v, wd_v, o_v, y_v, acc_v, hid_v,
            s_w, s_kv, s_o):
    cp = pltpu.make_async_copy

    def wait_all(buf, sem):
        cp(buf, buf, sem).wait()

    def c_ffn(a, r):
        i = (slice(None), ds(pl.multiple_of(16 * r, 16), 16))
        return cp((wg_h, wu_h, wd_h)[a].at[i], (wg_v, wu_v, wd_v)[a].at[i], s_w.at[a])

    def c_wq(a, r):
        n = NW * a + r
        i = (slice(None), ds(pl.multiple_of((n >> 2) * 8, 8), 8), ds(pl.multiple_of((n & 3) * 1024, 1024), 1024))
        return cp(wq_h.at[i], wq_v.at[i], s_w.at[3])

    def c_wo(a, r):
        i = (ds(2 * a, 2), ds(pl.multiple_of(LATE + 16 * r, 16), 16))
        return cp(wo_h.at[i], wo_v.at[i], s_w.at[4])

    weights = {HI: ((c_wq, 0), (c_ffn, 1), (c_wo, 0), (c_wq, 2)),
               LO: ((c_ffn, 0), (c_wq, 1), (c_ffn, 2), (c_wo, 1))}

    def start_w(pr, j, r):
        c, a = weights[pr][j]
        if c is c_wq and a == 2:
            pl.when(r < NW - 1)(lambda: c(a, r).start(priority=pr))
        else:
            c(a, r).start(priority=pr)

    def start_kv(pr, j, r):
        t, s = 1 - pr, r // RPS
        src = (k_h, v_h)[t].at[0, ds((r // RG) * G + 2 * j, 2), ds(pl.multiple_of(SK - W + (r % RG) * CR, CR), CR)]
        dst = kv_v.at[s, t, ds(2 * j, 2), ds(pl.multiple_of((r % RPS) * CR, CR), CR)]
        cp(src, dst, s_kv.at[s % RING]).start(priority=pr)

    def rounds(lo, hi, hi_copy, lo_copy):
        def body(r, carry):
            for j in range(4):
                if hi_copy is not None:
                    hi_copy(j, r)
                lo_copy(j, r)
            return carry
        jax.lax.fori_loop(lo, hi, body, 0)

    def kv_rounds(lo, hi):
        rounds(lo, hi, lambda j, r: start_kv(HI, j, r), lambda j, r: start_kv(LO, j, r + AHEAD))

    blocks = _late_blocks()
    late = []
    for b, (g0, ng, r0, n) in enumerate(blocks):
        if ng > 1:
            idx = [(ds(g, 2), ds(r, 16)) for r in range(r0, r0 + n, 16) for g in range(g0, g0 + ng, 2)]
        else:
            idx = [(g0, ds(r, TINY)) for r in range(r0, r0 + n, TINY)]
        late += [cp(wo_h.at[i], wo_v.at[i], s_o.at[b]) for i in idx]
    n_hi = (len(late) - 4 * AHEAD) // 2 + 2
    late_hi = late[1:2 * n_hi:2]
    late_lo = late[0:2 * n_hi:2] + late[2 * n_hi:]

    rounds(0, AHEAD, None, lambda j, r: start_w(LO, j, r))
    copy_x = cp(x_h, x_v, s_w.at[5])
    copy_wr = cp(wr_h, wr_v, s_w.at[6])
    copy_x.start()
    copy_wr.start()
    rounds(0, NW - AHEAD, lambda j, r: start_w(HI, j, r), lambda j, r: start_w(LO, j, r + AHEAD))

    copy_x.wait()
    copy_wr.wait()
    x = x_v[0].astype(F32)
    mean = jnp.mean(x, axis=-1, keepdims=True)
    var = jnp.mean(jnp.square(x - mean), axis=-1, keepdims=True)
    xn_b = ((x - mean) / jnp.sqrt(var + 1e-5)).astype(BF16)
    xn = xn_b.astype(F32)
    xn8 = jnp.broadcast_to(xn_b, (8, D))
    route = jnp.sum(xn * wr_v[...].reshape(1, D).astype(F32), axis=-1, keepdims=True)
    y_v[...] = jnp.zeros((8, D), F32)
    acc_v[...] = jnp.zeros((8, D), F32)

    rounds(NW - AHEAD, NW, lambda j, r: start_w(HI, j, r), lambda j, r: start_kv(LO, j, r - (NW - AHEAD)))
    kv_rounds(0, LAG * RPS)
    for a, buf in enumerate((wg_v, wu_v, wd_v, wq_v, wo_v.at[:, ds(LATE, QO - LATE)])):
        wait_all(buf, s_w.at[a])

    row = jax.lax.broadcasted_iota(jnp.int32, (8, DH), 0)
    row_k = jax.lax.broadcasted_iota(jnp.int32, (8, KS), 0)

    def project(o8, g, h0, h1):
        lhs = jnp.concatenate([jnp.where(row == h, o8, 0.0) for h in range(h0, h1)], axis=1).astype(BF16)
        return jnp.dot(lhs, wo_v[g, ds(h0 * DH, (h1 - h0) * DH), :], preferred_element_type=F32)

    s_end = (NR - AHEAD - 1) // RPS - LAG + 1

    def step(s, carry):
        g, c = s // SPG, s % SPG
        kv_rounds(jnp.minimum((s + LAG) * RPS, NR - AHEAD), jnp.minimum((s + LAG + 1) * RPS, NR - AHEAD))

        @pl.when(s == s_end)
        def _():
            for i in range(4 * AHEAD):
                start_kv(HI, i % 4, NR - AHEAD + i // 4)
                late_lo[i].start(priority=LO)

        @pl.when(s == s_end + 1)
        def _():
            for i in range(max(len(late_hi), len(late_lo) - 4 * AHEAD)):
                if i < len(late_hi):
                    late_hi[i].start(priority=HI)
                if i + 4 * AHEAD < len(late_lo):
                    late_lo[i + 4 * AHEAD].start(priority=LO)

        def new_group():
            cols = ds(pl.multiple_of(g * QO, QO), QO)
            q = jnp.dot(xn8[:, :D // 2], wq_v[0, :, cols], preferred_element_type=F32)
            q = q + jnp.dot(xn8[:, D // 2:], wq_v[1, :, cols], preferred_element_type=F32)
            q8 = q[:, :DH]
            for h in range(1, G):
                q8 = jnp.where(row == h, q[:, h * DH:(h + 1) * DH], q8)
            return q8, jnp.full((8, DH), -jnp.inf, F32), jnp.zeros((8, DH), F32), jnp.zeros((8, DH), F32)

        q8, m, l, o = jax.lax.cond(c == 0, new_group, lambda: carry)

        @pl.when((g < 2) & (c == 2))
        def _():
            hid_v[...] = jax.nn.silu(jax.lax.dot_general(xn8, wg_v[g], _NT, preferred_element_type=F32))

        @pl.when((g < 2) & (c == 4))
        def _():
            hid_v[...] = hid_v[...] * jax.lax.dot_general(xn8, wu_v[g], _NT, preferred_element_type=F32)

        @pl.when((g < 2) & (c == 6))
        def _():
            y_v[...] += jnp.dot(hid_v[...].astype(BF16), wd_v[g], preferred_element_type=F32)

        wait_all(kv_v.at[s], s_kv.at[s % RING])
        q_b = q8.astype(BF16)
        sc = None
        for h in range(G):
            t = jax.lax.dot_general(q_b, kv_v[s, 0, h], _NT, preferred_element_type=F32)
            sc = t if sc is None else jnp.where(row_k == h, t, sc)
        sc = sc * DH ** -0.5
        m_new = jnp.maximum(m, jnp.max(sc, axis=-1, keepdims=True))
        m_sub = jnp.where(m_new == -jnp.inf, 0.0, m_new)
        alpha = jnp.exp(m - m_sub)
        p = jnp.exp(sc - jnp.concatenate([m_sub] * (KS // DH), axis=1))
        l = l * alpha + sum(p[:, i * DH:(i + 1) * DH] for i in range(KS // DH))
        p_b = p.astype(BF16)
        pv = None
        for h in range(G):
            t = jnp.dot(p_b, kv_v[s, 1, h], preferred_element_type=F32)
            pv = t if pv is None else jnp.where(row == h, t, pv)
        o = o * alpha + pv

        @pl.when(c == SPG - 1)
        def _():
            o8 = o / jnp.sum(l, axis=-1, keepdims=True)
            o_v[g] = o8
            acc_v[...] += project(o8, g, -(-LATE // DH), G)

        return q8, m_new, l, o

    zero = jnp.zeros((8, DH), F32)
    jax.lax.fori_loop(0, NS, step, (zero, zero, zero, zero))

    upd = xn * 0.0 + y_v[...] * jax.nn.sigmoid(route)
    gate = jax.nn.silu(xn + upd)
    o_first = o_v[0].astype(BF16).astype(F32)
    o_col = jnp.broadcast_to(o_first[0:1], (DH, DH)).T
    x8 = jnp.broadcast_to(x, (8, D))
    acc = acc_v[...]
    for b, (g0, ng, r0, n) in enumerate(blocks):
        wait_all(wo_v.at[ds(g0, ng), ds(r0, n)], s_o.at[b])
        if b < len(blocks) - len(VPU):
            for g in range(g0, g0 + ng):
                acc = acc + project(o_v[g], g, r0 // DH, r0 // DH + 1)
        else:
            coef = jnp.concatenate([o_col[r0:r0 + n]] * (D // DH), axis=1)
            prod = wo_v[0, ds(r0, n), :].astype(F32) * coef
            acc = acc + prod.reshape(n // 8, 8, D).sum(axis=0)
    s_out = jnp.sum(acc, axis=0, keepdims=True)

    res = x8 + jnp.broadcast_to(s_out, (8, D)) * gate
    out_ref[0] = res.astype(out_ref.dtype)[0:1]


@jax.jit
def pallas_recurrent_scan__sliding_block_cached__moe_arch_mod__decode_kernel(
    A_x: jax.Array,
    A_k_cache: jax.Array,
    A_v_cache: jax.Array,
    A_wq: jax.Array,
    A_wo: jax.Array,
    B_x: jax.Array,
    B_w_r: jax.Array,
    B_w_gate: jax.Array,
    B_w_up: jax.Array,
    B_w_down: jax.Array,
):
    del B_x
    hbm = pl.BlockSpec(memory_space=pltpu.HBM)
    dma = pltpu.SemaphoreType.DMA
    ffn = (2, F // 2, D)
    return pl.pallas_call(
        _kernel,
        out_shape=jax.ShapeDtypeStruct((1, 1, D), BF16),
        in_specs=[hbm] * 9,
        out_specs=pl.BlockSpec(memory_space=pltpu.VMEM),
        scratch_shapes=[
            pltpu.VMEM((1, 1, D), BF16),
            pltpu.VMEM((D,), BF16),
            pltpu.VMEM((2, D // 2, NH * DH), BF16),
            pltpu.VMEM((NS, 2, G, KS, DH), BF16),
            pltpu.VMEM((NG, QO, D), BF16),
            pltpu.VMEM(ffn, BF16),
            pltpu.VMEM(ffn, BF16),
            pltpu.VMEM(ffn, BF16),
            pltpu.VMEM((NG, 8, DH), F32),
            pltpu.VMEM((8, D), F32),
            pltpu.VMEM((8, D), F32),
            pltpu.VMEM((8, F // 2), F32),
            dma((7,)), dma((RING,)), dma((len(_late_blocks()),)),
        ],
        compiler_params=pltpu.CompilerParams(
            vmem_limit_bytes=100 * 1024 * 1024,
            disable_semaphore_checks=True,
        ),
    )(A_x, A_k_cache, A_v_cache, A_wq.reshape(2, D // 2, NH * DH), A_wo.reshape(NG, QO, D), B_w_r,
      B_w_gate.T.reshape(ffn), B_w_up.T.reshape(ffn), B_w_down.reshape(ffn))
```

```python
import jax
import jax.numpy as jnp
import jax.experimental.pallas as pl
import jax.experimental.pallas.tpu as pltpu

D = 512
NH = 32
DH = 128
SK = 32768
W = min(4096, max(256, SK // 4))
F = 1376

P = 16
G = 16
NG = NH // G
CR = 64
KS = 4 * CR
SPG = W // KS
NS = NG * SPG
NW = 8
NO = 3
AHEAD = 27
LAG = 2
RING = 8
TINY = 8
ALONE = 22
TAIL_MXU = (((0, 2), (2, 2), (0, DH)), ((0, 2), (1, 1), (0, DH)))
TAIL_VPU = (((1, 1), (0, 1), (0, 64)), ((1, 1), (0, 1), (64, 64)),
            ((0, 1), (0, 1), (0, 80)), ((0, 1), (0, 1), (80, 32)), ((0, 1), (0, 1), (112, 16)))

BF16 = jnp.bfloat16
F32 = jnp.float32
_NT = (((1,), (1,)), ((), ()))
HI, LO = 0, 1
ds = pl.ds


def _aligned(v, n):
    return v if isinstance(v, int) else pl.multiple_of(v, n)


def _kernel(x_h, k_h, v_h, wq_h, wo_h, wr_h, wg_h, wu_h, wd_h, out_ref,
            x_v, wr_v, wq_v, kv_v, wo_v, f_v, q_v, sc_v, m_v, o_v, y_v, hid_v,
            s_w, s_kv, s_o):
    cp = pltpu.make_async_copy

    def wait_all(buf, sem):
        cp(buf, buf, sem).wait()

    def start_ffn(pr, a, r):
        i = (slice(None), ds(_aligned(16 * r, 16), 16))
        cp((wg_h, wu_h, wd_h)[a].at[i], f_v.at[(a,) + i], s_w.at[0]).start(priority=pr)

    def start_w(pr, s, i):
        if pr == HI:
            ix = (slice(None), ds(_aligned(64 * (0, 2, 1, 3)[i % 4] + 8 * s, 8), 8), ds(1024 * (i // 4), 1024))
            cp(wq_h.at[ix], wq_v.at[ix], s_w.at[1]).start(priority=pr)
        elif i < 15:
            start_ffn(pr, i % 3, 5 * s + i // 3)
        elif isinstance(s, int):
            start_ffn(pr, s // 3, 40 + s % 3)
        else:
            for a in range(3):
                pl.when((s >= 3 * a) & (s < 3 * a + 3))(lambda a=a: start_ffn(pr, a, 40 + s - 3 * a))

    def start_kv(t):
        def start(pr, s, i):
            h, r = 8 * (1 - pr) + 2 * (i % 4), (i // 4) * CR
            src = (k_h, v_h)[t].at[0, ds((s // SPG) * G + h, 2), ds(_aligned(SK - W + (s % SPG) * KS + r, CR), CR)]
            cp(src, kv_v.at[t, s, ds(h, 2), ds(r, CR)], s_kv.at[s % RING]).start(priority=pr)
        return start

    def start_wo(pr, s, i):
        ix = (slice(None), 2 * (1 - pr) + i % 2, ds((NO - s) * DH + (i // 2) * 16, 16))
        cp(wo_h.at[ix], wo_v.at[ix], s_o.at[s]).start(priority=pr)

    tail = []
    for b, (_, (q0, nq), (r0, n)) in enumerate(TAIL_MXU):
        tail += [((slice(None), q, ds(r, 16)), NO + b) for r in range(r0, r0 + n, 16) for q in range(q0, q0 + nq)]
    for b, ((a, _), (q, _), (r0, n)) in enumerate(TAIL_VPU):
        tail += [((a, q, ds(r, TINY)), NO + len(TAIL_MXU) + b) for r in range(r0, r0 + n, TINY)]
    n_hi = (len(tail) - ALONE) // 2
    tail = {HI: tail[1:2 * n_hi:2], LO: tail[0:2 * n_hi:2] + tail[2 * n_hi:]}

    def start_nth(pr, n):
        s, i = divmod(n, P)
        for start, steps in ((start_w, NW), (start_kv(0), NS), (start_kv(1), NS), (start_wo, NO)):
            if s < steps:
                return start(pr, s, i)
            s -= steps
        if s * P + i < len(tail[pr]):
            ix, b = tail[pr][s * P + i]
            cp(wo_h.at[ix], wo_v.at[ix], s_o.at[b]).start(priority=pr)

    def pairs_at(n0, n1):
        for n in range(n0, n1):
            start_nth(HI, n)
            start_nth(LO, n + AHEAD)

    def pairs_of(start, s):
        for i in range(P):
            start(HI, s, i)
            start(LO, s + (i + AHEAD) // P, (i + AHEAD) % P)

    start_nth(LO, 0)
    start_nth(HI, 0)
    for n in range(1, AHEAD + 1):
        start_nth(LO, n)
    pairs_at(1, P)
    copy_x = cp(x_h, x_v, s_w.at[2])
    copy_wr = cp(wr_h, wr_v, s_w.at[3])
    copy_x.start()
    copy_wr.start()
    start_ffn(HI, 2, 42)
    jax.lax.fori_loop(1, NW - 2, lambda s, _: pairs_of(start_w, s), None)
    pairs_at((NW - 2) * P, NW * P)

    copy_x.wait()
    copy_wr.wait()
    x = x_v[0].astype(F32)
    mean = jnp.mean(x, axis=-1, keepdims=True)
    var = jnp.mean(jnp.square(x - mean), axis=-1, keepdims=True)
    xn_b = ((x - mean) / jnp.sqrt(var + 1e-5)).astype(BF16)
    xn = xn_b.astype(F32)
    xn8 = jnp.broadcast_to(xn_b, (8, D))
    route = jnp.sum(xn * wr_v[...].reshape(1, D).astype(F32), axis=-1, keepdims=True)
    y_v[...] = jnp.zeros((8, D), F32)

    row = jax.lax.broadcasted_iota(jnp.int32, (8, DH), 0)
    row_k = jax.lax.broadcasted_iota(jnp.int32, (8, KS), 0)

    def scores(s):
        g, c = s // SPG, s % SPG

        @pl.when(s == 0)
        def _():
            wait_all(f_v, s_w.at[0])
            wait_all(wq_v, s_w.at[1])

        @pl.when(c == 0)
        def _():
            for u in range(2):
                cols = ds(pl.multiple_of((2 * g + u) * 8 * DH, 8 * DH), 8 * DH)
                q = jnp.dot(xn8[:, :D // 2], wq_v[0, :, cols], preferred_element_type=F32)
                q = q + jnp.dot(xn8[:, D // 2:], wq_v[1, :, cols], preferred_element_type=F32)
                q8 = q[:, :DH]
                for h in range(1, 8):
                    q8 = jnp.where(row == h, q[:, h * DH:(h + 1) * DH], q8)
                q_v[u] = q8
                m_v[g, u] = jnp.full((8, KS), -jnp.inf, F32)

        @pl.when(c == 3)
        def _():
            hid_v[...] = jax.nn.silu(jax.lax.dot_general(xn8, f_v[0, g], _NT, preferred_element_type=F32))

        @pl.when(c == 5)
        def _():
            hid_v[...] = hid_v[...] * jax.lax.dot_general(xn8, f_v[1, g], _NT, preferred_element_type=F32)

        @pl.when(c == 7)
        def _():
            y_v[...] += jnp.dot(hid_v[...].astype(BF16), f_v[2, g], preferred_element_type=F32)

        wait_all(kv_v.at[0, s], s_kv.at[s % RING])
        for u in range(2):
            q_b = q_v[u].astype(BF16)
            sc = None
            for h in range(8):
                t = jax.lax.dot_general(q_b, kv_v[0, s, 8 * u + h], _NT, preferred_element_type=F32)
                sc = t if sc is None else jnp.where(row_k == h, t, sc)
            sc = sc * DH ** -0.5
            sc_v[s, u] = sc
            m_v[g, u] = jnp.maximum(m_v[g, u], sc)

    def values(s, carry):
        g, c = s // SPG, s % SPG
        wait_all(kv_v.at[1, s], s_kv.at[s % RING])
        new = []
        for u, (l, o) in enumerate(carry):
            p = jnp.exp(sc_v[s, u] - jnp.max(m_v[g, u], axis=-1, keepdims=True))
            p_b = p.astype(BF16)
            pv = None
            for h in range(8):
                t = jnp.dot(p_b, kv_v[1, s, 8 * u + h], preferred_element_type=F32)
                pv = t if pv is None else jnp.where(row == h, t, pv)
            new.append((jnp.where(c == 0, 0.0, l) + p, jnp.where(c == 0, 0.0, o) + pv))

        @pl.when(c == SPG - 1)
        def _():
            for u, (l, o) in enumerate(new):
                o_v[2 * g + u] = o / jnp.sum(l, axis=-1, keepdims=True)

        return tuple(new)

    def step(n, carry):
        pl.when(n < NS - 2)(lambda: pairs_of(start_kv(0), n))
        pl.when((n >= NS) & (n < 2 * NS - 2))(lambda: pairs_of(start_kv(1), n - NS))
        for e0, e1 in ((NS - 2, NS - 1), (NS - 1, NS), (2 * NS - 2, 2 * NS - 1), (2 * NS - 1, 2 * NS),
                       (2 * NS, 2 * NS + 1), (2 * NS + 1, 2 * NS + NO)):
            pl.when(n == e0)(lambda e0=e0, e1=e1: pairs_at((NW + e0) * P, (NW + e1) * P))
        pl.when((n >= LAG) & (n < NS + LAG))(lambda: scores(n - LAG))
        return jax.lax.cond(n >= NS + LAG, lambda: values(n - NS - LAG, carry), lambda: carry)

    jax.lax.fori_loop(0, 2 * NS + LAG, step, ((jnp.zeros((8, KS), F32), jnp.zeros((8, DH), F32)),) * 2)
    n0 = (NW + 2 * NS + NO) * P
    pairs_at(n0, n0 + max(len(tail[HI]), len(tail[LO]) - AHEAD))

    def project(a, q, b):
        lhs = jnp.where(row == 4 * (q % 2) + b, o_v[2 * a + q // 2], 0.0).astype(BF16)
        return jnp.dot(lhs, wo_v[a, q, ds(_aligned(b * DH, DH), DH), :], preferred_element_type=F32)

    def block(s, acc):
        wait_all(wo_v.at[:, :, ds(pl.multiple_of((NO - s) * DH, DH), DH)], s_o.at[s])
        for a in range(2):
            for q in range(4):
                acc = acc + project(a, q, NO - s)
        return acc

    upd = xn * 0.0 + y_v[...] * jax.nn.sigmoid(route)
    gate = jax.nn.silu(xn + upd)
    acc = jax.lax.fori_loop(0, NO, block, jnp.zeros((8, D), F32))
    o_col = [jnp.broadcast_to(o_v[2 * a].astype(BF16).astype(F32)[0:1], (DH, DH)).T for a in range(2)]
    x8 = jnp.broadcast_to(x, (8, D))
    for b, ((a0, na), (q0, nq), (r0, n)) in enumerate(TAIL_MXU + TAIL_VPU):
        wait_all(wo_v.at[ds(a0, na), ds(q0, nq), ds(r0, n)], s_o.at[NO + b])
        if b < len(TAIL_MXU):
            for a in range(a0, a0 + na):
                for q in range(q0, q0 + nq):
                    acc = acc + project(a, q, 0)
        else:
            coef = jnp.concatenate([o_col[a0][r0:r0 + n]] * (D // DH), axis=1)
            prod = wo_v[a0, q0, ds(r0, n), :].astype(F32) * coef
            acc = acc + prod.reshape(n // 8, 8, D).sum(axis=0)
    s_out = jnp.sum(acc, axis=0, keepdims=True)

    res = x8 + jnp.broadcast_to(s_out, (8, D)) * gate
    out_ref[0] = res.astype(out_ref.dtype)[0:1]


@jax.jit
def pallas_recurrent_scan__sliding_block_cached__moe_arch_mod__decode_kernel(
    A_x: jax.Array,
    A_k_cache: jax.Array,
    A_v_cache: jax.Array,
    A_wq: jax.Array,
    A_wo: jax.Array,
    B_x: jax.Array,
    B_w_r: jax.Array,
    B_w_gate: jax.Array,
    B_w_up: jax.Array,
    B_w_down: jax.Array,
):
    del B_x
    hbm = pl.BlockSpec(memory_space=pltpu.HBM)
    dma = pltpu.SemaphoreType.DMA
    wq_shape, wo_shape, ffn_shape = (2, D // 2, NH * DH), (2, 4, 4 * DH, D), (2, F // 2, D)
    return pl.pallas_call(
        _kernel,
        out_shape=jax.ShapeDtypeStruct((1, 1, D), BF16),
        in_specs=[hbm] * 9,
        out_specs=pl.BlockSpec(memory_space=pltpu.VMEM),
        scratch_shapes=[
            pltpu.VMEM((1, 1, D), BF16),
            pltpu.VMEM((D,), BF16),
            pltpu.VMEM(wq_shape, BF16),
            pltpu.VMEM((2, NS, G, KS, DH), BF16),
            pltpu.VMEM(wo_shape, BF16),
            pltpu.VMEM((3,) + ffn_shape, BF16),
            pltpu.VMEM((2, 8, DH), F32),
            pltpu.VMEM((NS, 2, 8, KS), F32),
            pltpu.VMEM((NG, 2, 8, KS), F32),
            pltpu.VMEM((2 * NG, 8, DH), F32),
            pltpu.VMEM((8, D), F32),
            pltpu.VMEM((8, F // 2), F32),
            dma((4,)), dma((RING,)), dma((NO + len(TAIL_MXU) + len(TAIL_VPU),)),
        ],
        compiler_params=pltpu.CompilerParams(
            vmem_limit_bytes=100 * 1024 * 1024,
            disable_semaphore_checks=True,
        ),
    )(A_x, A_k_cache, A_v_cache, A_wq.reshape(wq_shape), A_wo.reshape(wo_shape), B_w_r,
      B_w_gate.T.reshape(ffn_shape), B_w_up.T.reshape(ffn_shape), B_w_down.reshape(ffn_shape))
```

```python
import jax
import jax.numpy as jnp
import jax.experimental.pallas as pl
import jax.experimental.pallas.tpu as pltpu

D = 512
NH = 32
DH = 128
SK = 32768
W = min(4096, max(256, SK // 4))
F = 1376

P = 16
G = 16
NG = NH // G
CR = 64
KS = 4 * CR
SPG = W // KS
NS = NG * SPG
NW = 8
NO = 3
AHEAD = 27
LAG = 2
RING = 8
TINY = 8
ALONE = 30
TAIL_MXU = (((0, 2), (2, 2), (0, DH)), ((0, 2), (1, 1), (0, DH)))
TAIL_VPU = (((1, 1), (0, 1), (0, 64)), ((1, 1), (0, 1), (64, 64)),
            ((0, 1), (0, 1), (0, 80)), ((0, 1), (0, 1), (80, 32)), ((0, 1), (0, 1), (112, 16)))

BF16 = jnp.bfloat16
F32 = jnp.float32
_NT = (((1,), (1,)), ((), ()))
HI, LO = 0, 1
ds = pl.ds


def _aligned(v, n):
    return v if isinstance(v, int) else pl.multiple_of(v, n)


def _kernel(x_h, k_h, v_h, wq_h, wo_h, wr_h, wg_h, wu_h, wd_h, out_ref,
            x_v, wr_v, wq_v, kv_v, wo_v, f_v, q_v, sc_v, m_v, o_v, y_v, hid_v,
            s_w, s_kv, s_o):
    cp = pltpu.make_async_copy

    def wait_all(buf, sem):
        cp(buf, buf, sem).wait()

    def start_ffn(pr, a, r):
        i = (slice(None), ds(_aligned(16 * r, 16), 16))
        cp((wg_h, wu_h, wd_h)[a].at[i], f_v.at[(a,) + i], s_w.at[0]).start(priority=pr)

    def start_w(pr, s, i):
        if pr == HI:
            ix = (slice(None), ds(_aligned(64 * (0, 2, 1, 3)[i % 4] + 8 * s, 8), 8), ds(1024 * (i // 4), 1024))
            cp(wq_h.at[ix], wq_v.at[ix], s_w.at[1]).start(priority=pr)
        elif i < 15:
            start_ffn(pr, i % 3, 5 * s + i // 3)
        elif isinstance(s, int):
            start_ffn(pr, s // 3, 40 + s % 3)
        else:
            for a in range(3):
                pl.when((s >= 3 * a) & (s < 3 * a + 3))(lambda a=a: start_ffn(pr, a, 40 + s - 3 * a))

    def start_kv(t):
        def start(pr, s, i):
            h, r = 8 * (1 - pr) + 2 * (i % 4), (i // 4) * CR
            src = (k_h, v_h)[t].at[0, ds((s // SPG) * G + h, 2), ds(_aligned(SK - W + (s % SPG) * KS + r, CR), CR)]
            cp(src, kv_v.at[t, s, ds(h, 2), ds(r, CR)], s_kv.at[s % RING]).start(priority=pr)
        return start

    def start_wo(pr, s, i):
        ix = (slice(None), 2 * (1 - pr) + i % 2, ds((NO - s) * DH + (i // 2) * 16, 16))
        cp(wo_h.at[ix], wo_v.at[ix], s_o.at[s]).start(priority=pr)

    tail = []
    for b, (_, (q0, nq), (r0, n)) in enumerate(TAIL_MXU):
        tail += [((slice(None), q, ds(r, 16)), NO + b) for r in range(r0, r0 + n, 16) for q in range(q0, q0 + nq)]
    for b, ((a, _), (q, _), (r0, n)) in enumerate(TAIL_VPU):
        tail += [((a, q, ds(r, TINY)), NO + len(TAIL_MXU) + b) for r in range(r0, r0 + n, TINY)]
    n_hi = (len(tail) - ALONE) // 2
    tail = {HI: tail[1:2 * n_hi:2], LO: tail[0:2 * n_hi:2] + tail[2 * n_hi:]}

    def start_nth(pr, n):
        s, i = divmod(n, P)
        for start, steps in ((start_w, NW), (start_kv(0), NS), (start_kv(1), NS), (start_wo, NO)):
            if s < steps:
                return start(pr, s, i)
            s -= steps
        if s * P + i < len(tail[pr]):
            ix, b = tail[pr][s * P + i]
            cp(wo_h.at[ix], wo_v.at[ix], s_o.at[b]).start(priority=pr)

    def pairs_at(n0, n1):
        for n in range(n0, n1):
            start_nth(HI, n)
            start_nth(LO, n + AHEAD)

    def pairs_of(start, s):
        for i in range(P):
            start(HI, s, i)
            start(LO, s + (i + AHEAD) // P, (i + AHEAD) % P)

    copy_x = cp(x_h, x_v, s_w.at[2])
    copy_wr = cp(wr_h, wr_v, s_w.at[3])
    start_nth(LO, 0)
    start_ffn(HI, 2, 42)
    start_nth(LO, 1)
    copy_x.start(priority=HI)
    start_nth(LO, 2)
    copy_wr.start(priority=LO)
    for n in range(3, AHEAD):
        start_nth(LO, n)
    pairs_at(0, P)
    jax.lax.fori_loop(1, NW - 2, lambda s, _: pairs_of(start_w, s), None)
    pairs_at((NW - 2) * P, NW * P)

    copy_x.wait()
    copy_wr.wait()
    x = x_v[0].astype(F32)
    mean = jnp.mean(x, axis=-1, keepdims=True)
    var = jnp.mean(jnp.square(x - mean), axis=-1, keepdims=True)
    xn_b = ((x - mean) / jnp.sqrt(var + 1e-5)).astype(BF16)
    xn = xn_b.astype(F32)
    xn8 = jnp.broadcast_to(xn_b, (8, D))
    route = jnp.sum(xn * wr_v[...].reshape(1, D).astype(F32), axis=-1, keepdims=True)
    y_v[...] = jnp.zeros((8, D), F32)

    row = jax.lax.broadcasted_iota(jnp.int32, (8, DH), 0)
    row_k = jax.lax.broadcasted_iota(jnp.int32, (8, KS), 0)

    def scores(s):
        g, c = s // SPG, s % SPG

        @pl.when(s == 0)
        def _():
            wait_all(f_v, s_w.at[0])
            wait_all(wq_v, s_w.at[1])

        @pl.when(c == 0)
        def _():
            for u in range(2):
                cols = ds(pl.multiple_of((2 * g + u) * 8 * DH, 8 * DH), 8 * DH)
                q = jnp.dot(xn8[:, :D // 2], wq_v[0, :, cols], preferred_element_type=F32)
                q = q + jnp.dot(xn8[:, D // 2:], wq_v[1, :, cols], preferred_element_type=F32)
                q8 = q[:, :DH]
                for h in range(1, 8):
                    q8 = jnp.where(row == h, q[:, h * DH:(h + 1) * DH], q8)
                q_v[u] = q8
                m_v[g, u] = jnp.full((8, KS), -jnp.inf, F32)

        @pl.when(c == 3)
        def _():
            hid_v[...] = jax.nn.silu(jax.lax.dot_general(xn8, f_v[0, g], _NT, preferred_element_type=F32))

        @pl.when(c == 5)
        def _():
            hid_v[...] = hid_v[...] * jax.lax.dot_general(xn8, f_v[1, g], _NT, preferred_element_type=F32)

        @pl.when(c == 7)
        def _():
            y_v[...] += jnp.dot(hid_v[...].astype(BF16), f_v[2, g], preferred_element_type=F32)

        wait_all(kv_v.at[0, s], s_kv.at[s % RING])
        for u in range(2):
            q_b = q_v[u].astype(BF16)
            sc = None
            for h in range(8):
                t = jax.lax.dot_general(q_b, kv_v[0, s, 8 * u + h], _NT, preferred_element_type=F32)
                sc = t if sc is None else jnp.where(row_k == h, t, sc)
            sc = sc * DH ** -0.5
            sc_v[s, u] = sc
            m_v[g, u] = jnp.maximum(m_v[g, u], sc)

    def values(s, carry):
        g, c = s // SPG, s % SPG
        wait_all(kv_v.at[1, s], s_kv.at[s % RING])
        new = []
        for u, (l, o) in enumerate(carry):
            p = jnp.exp(sc_v[s, u] - jnp.max(m_v[g, u], axis=-1, keepdims=True))
            p_b = p.astype(BF16)
            pv = None
            for h in range(8):
                t = jnp.dot(p_b, kv_v[1, s, 8 * u + h], preferred_element_type=F32)
                pv = t if pv is None else jnp.where(row == h, t, pv)
            new.append((jnp.where(c == 0, 0.0, l) + p, jnp.where(c == 0, 0.0, o) + pv))

        @pl.when(c == SPG - 1)
        def _():
            for u, (l, o) in enumerate(new):
                o_v[2 * g + u] = o / jnp.sum(l, axis=-1, keepdims=True)

        return tuple(new)

    def step(n, carry):
        pl.when(n < NS - 2)(lambda: pairs_of(start_kv(0), n))
        pl.when((n >= NS) & (n < 2 * NS - 2))(lambda: pairs_of(start_kv(1), n - NS))
        for e0, e1 in ((NS - 2, NS - 1), (NS - 1, NS), (2 * NS - 2, 2 * NS - 1), (2 * NS - 1, 2 * NS),
                       (2 * NS, 2 * NS + 1), (2 * NS + 1, 2 * NS + NO)):
            pl.when(n == e0)(lambda e0=e0, e1=e1: pairs_at((NW + e0) * P, (NW + e1) * P))
        pl.when((n >= LAG) & (n < NS + LAG))(lambda: scores(n - LAG))
        return jax.lax.cond(n >= NS + LAG, lambda: values(n - NS - LAG, carry), lambda: carry)

    jax.lax.fori_loop(0, 2 * NS + LAG, step, ((jnp.zeros((8, KS), F32), jnp.zeros((8, DH), F32)),) * 2)
    n0 = (NW + 2 * NS + NO) * P
    pairs_at(n0, n0 + max(len(tail[HI]), len(tail[LO]) - AHEAD))

    def project(a, q, b):
        lhs = jnp.where(row == 4 * (q % 2) + b, o_v[2 * a + q // 2], 0.0).astype(BF16)
        return jnp.dot(lhs, wo_v[a, q, ds(_aligned(b * DH, DH), DH), :], preferred_element_type=F32)

    def block(s, acc):
        wait_all(wo_v.at[:, :, ds(pl.multiple_of((NO - s) * DH, DH), DH)], s_o.at[s])
        for a in range(2):
            for q in range(4):
                acc = acc + project(a, q, NO - s)
        return acc

    upd = xn * 0.0 + y_v[...] * jax.nn.sigmoid(route)
    gate = jax.nn.silu(xn + upd)
    acc = jax.lax.fori_loop(0, NO, block, jnp.zeros((8, D), F32))
    o_col = [jnp.broadcast_to(o_v[2 * a].astype(BF16).astype(F32)[0:1], (DH, DH)).T for a in range(2)]
    x8 = jnp.broadcast_to(x, (8, D))
    for b, ((a0, na), (q0, nq), (r0, n)) in enumerate(TAIL_MXU + TAIL_VPU):
        wait_all(wo_v.at[ds(a0, na), ds(q0, nq), ds(r0, n)], s_o.at[NO + b])
        if b < len(TAIL_MXU):
            for a in range(a0, a0 + na):
                for q in range(q0, q0 + nq):
                    acc = acc + project(a, q, 0)
        else:
            coef = jnp.concatenate([o_col[a0][r0:r0 + n]] * (D // DH), axis=1)
            prod = wo_v[a0, q0, ds(r0, n), :].astype(F32) * coef
            acc = acc + prod.reshape(n // 8, 8, D).sum(axis=0)
    s_out = jnp.sum(acc, axis=0, keepdims=True)

    res = x8 + jnp.broadcast_to(s_out, (8, D)) * gate
    out_ref[0] = res.astype(out_ref.dtype)[0:1]


@jax.jit
def pallas_recurrent_scan__sliding_block_cached__moe_arch_mod__decode_kernel(
    A_x: jax.Array,
    A_k_cache: jax.Array,
    A_v_cache: jax.Array,
    A_wq: jax.Array,
    A_wo: jax.Array,
    B_x: jax.Array,
    B_w_r: jax.Array,
    B_w_gate: jax.Array,
    B_w_up: jax.Array,
    B_w_down: jax.Array,
):
    del B_x
    hbm = pl.BlockSpec(memory_space=pltpu.HBM)
    dma = pltpu.SemaphoreType.DMA
    wq_shape, wo_shape, ffn_shape = (2, D // 2, NH * DH), (2, 4, 4 * DH, D), (2, F // 2, D)
    return pl.pallas_call(
        _kernel,
        out_shape=jax.ShapeDtypeStruct((1, 1, D), BF16),
        in_specs=[hbm] * 9,
        out_specs=pl.BlockSpec(memory_space=pltpu.VMEM),
        scratch_shapes=[
            pltpu.VMEM((1, 1, D), BF16),
            pltpu.VMEM((D,), BF16),
            pltpu.VMEM(wq_shape, BF16),
            pltpu.VMEM((2, NS, G, KS, DH), BF16),
            pltpu.VMEM(wo_shape, BF16),
            pltpu.VMEM((3,) + ffn_shape, BF16),
            pltpu.VMEM((2, 8, DH), F32),
            pltpu.VMEM((NS, 2, 8, KS), F32),
            pltpu.VMEM((NG, 2, 8, KS), F32),
            pltpu.VMEM((2 * NG, 8, DH), F32),
            pltpu.VMEM((8, D), F32),
            pltpu.VMEM((8, F // 2), F32),
            dma((4,)), dma((RING,)), dma((NO + len(TAIL_MXU) + len(TAIL_VPU),)),
        ],
        compiler_params=pltpu.CompilerParams(
            vmem_limit_bytes=100 * 1024 * 1024,
            disable_semaphore_checks=True,
        ),
    )(A_x, A_k_cache, A_v_cache, A_wq.reshape(wq_shape), A_wo.reshape(wo_shape), B_w_r,
      B_w_gate.T.reshape(ffn_shape), B_w_up.T.reshape(ffn_shape), B_w_down.reshape(ffn_shape))
```
